```python
import jax
import jax.numpy as jnp

def _softmax(x, axis=-1):
    return jax.nn.softmax(x, axis=axis)
def _gelu(x):
    return jax.nn.gelu(x, approximate=True)
def _silu(x):
    return jax.nn.silu(x)
def _sigmoid(x):
    return jax.nn.sigmoid(x)
def _layernorm(x, axis=-1, eps=1e-5):
    m = jnp.mean(x, axis=axis, keepdims=True)
    v = jnp.var(x, axis=axis, keepdims=True)
    return (x - m) / jnp.sqrt(v + eps)
def _scatter_add(tgt, idx, src, axis=0):
    return tgt.at[idx].add(src)
def _segment_sum(src, seg, n):
    return jax.ops.segment_sum(src, seg, n)
class _Rng:
    def __init__(self, key):
        self._k = key
    def _next(self):
        self._k, sub = jax.random.split(self._k)
        return sub
    def normal(self, shape):
        return jax.random.normal(self._next(), shape, dtype=jnp.bfloat16)
    def randint(self, lo, hi, shape):
        return jax.random.randint(self._next(), shape, lo, hi, dtype=jnp.int32)
    def uniform(self, shape, lo=0.0, hi=1.0):
        return jax.random.uniform(self._next(), shape, jnp.bfloat16, lo, hi)
    def permutation(self, n):
        return jax.random.permutation(self._next(), n)


kernel_name = 'gated_mix__mha_block_cached__moe_arch_mod__decode'

def setup_inputs():
    _rng = _Rng(jax.random.key(int.from_bytes(__import__("os").urandom(4), "little")))
    _w = (lambda a: (lambda t: t.astype(jnp.bfloat16) if jnp.issubdtype(t.dtype, jnp.floating) else t)(jnp.asarray(a)))
    def _A_setup():
        B, Sq, D = 4, 1, 1024
        H, Sk, Dh = 32, 8192, 128
        return {
            "x": _w((lambda *s: _rng.normal(s) * 0.05)(B, Sq, D)),
            "k_cache": _w((lambda *s: _rng.normal(s) * 0.05)(B, H, Sk, Dh)),
            "v_cache": _w((lambda *s: _rng.normal(s) * 0.05)(B, H, Sk, Dh)),
            "wq": _w((lambda *s: _rng.normal(s) * 0.05)(D, H * Dh) * (D ** -0.5)),
            "wo": _w((lambda *s: _rng.normal(s) * 0.05)(H * Dh, D) * ((H * Dh) ** -0.5)),
        }
    _A_in = _A_setup()

    def _B_setup():
        B, S, D, F, C = 4, 1, 1024, 3584, 1
        return {
            "x": _w((lambda *s: _rng.normal(s) * 0.05)(B, S, D)),
            "w_r": _w((lambda *s: _rng.normal(s) * 0.05)(D)),
            "w_gate": _w((lambda *s: _rng.normal(s) * 0.05)(D, F)),
            "w_up": _w((lambda *s: _rng.normal(s) * 0.05)(D, F)),
            "w_down": _w((lambda *s: _rng.normal(s) * 0.05)(F, D)),
        }
    _B_in = _B_setup()

    return {
        "A_x": _A_in["x"],
        "A_k_cache": _A_in["k_cache"],
        "A_v_cache": _A_in["v_cache"],
        "A_wq": _A_in["wq"],
        "A_wo": _A_in["wo"],
        "B_x": _B_in["x"],
        "B_w_r": _B_in["w_r"],
        "B_w_gate": _B_in["w_gate"],
        "B_w_up": _B_in["w_up"],
        "B_w_down": _B_in["w_down"],
        "gate_w": _w((lambda *s: _rng.normal(s) * 0.05)(1024)),
    }

def reference(A_x, A_k_cache, A_v_cache, A_wq, A_wo, B_x, B_w_r, B_w_gate, B_w_up, B_w_down, gate_w):
    def _A_ref(x, k_cache, v_cache, wq, wo):
        B, Sq, D = x.shape
        H, Dh = 32, 128
        q = (lambda x, *d: x.transpose(*d))((x @ wq).reshape(B, Sq, H, Dh), 0, 2, 1, 3)
        scores = jnp.einsum("bhqd,bhkd->bhqk", q, k_cache) * (Dh ** -0.5)
        p = _softmax(scores, axis=-1)
        o = jnp.einsum("bhqk,bhkd->bhqd", p, v_cache)
        return (lambda x, *d: x.transpose(*d))(o, 0, 2, 1, 3).reshape(B, Sq, H * Dh) @ wo

    def _B_ref(x, w_r, w_gate, w_up, w_down):
        B, S, D = x.shape
        C = 1
        r = x @ w_r
        idx = jnp.argsort(-r, axis=-1)[:, :C]
        idx_e = jnp.repeat(idx.reshape(B, C, 1), D, axis=2)
        x_sel = jnp.take_along_axis(x, idx_e, axis=1)
        g = _silu(x_sel @ w_gate)
        u = x_sel @ w_up
        y = (g * u) @ w_down
        r_sel = _sigmoid(jnp.take_along_axis(r, idx, axis=1))
        y = y * r_sel.reshape(B, C, 1)
        b_off = (jnp.arange(B) * S).reshape(B, 1)
        flat_idx = (idx + b_off).reshape(B * C)
        zero = (x * 0.0).reshape(B * S, D)
        upd = _scatter_add(zero, flat_idx, y.reshape(B * C, D), axis=0)
        return x + upd.reshape(B, S, D)

    x = A_x
    g = _sigmoid((x * gate_w).sum(-1, keepdims=True))
    a = _A_ref(x, A_k_cache, A_v_cache, A_wq, A_wo)
    b = _B_ref(x, B_w_r, B_w_gate, B_w_up, B_w_down)
    return g * a + (1 - g) * b
```

```python
import jax
import jax.numpy as jnp
import jax.experimental.pallas as pl
import jax.experimental.pallas.tpu as pltpu

B, D, H, SK, DH, F = 4, 1024, 32, 8192, 128, 3584
NBUF = 4
NPAIR = B * H
f32 = jnp.float32
bf16 = jnp.bfloat16


def _kernel(x_ref, wr_ref, gw_ref, k_hbm, v_hbm, wq_hbm, wo_hbm, wg_hbm, wu_hbm, wd_hbm,
            o_ref,
            kbuf, vbuf, wq_v, wo_v, wg_v, wu_v, wd_v, q_v, oh_v, acc_v, b_v,
            ksem, vsem, wsem):
    def kcopy(i, slot):
        return pltpu.make_async_copy(k_hbm.at[i % B, i // B], kbuf.at[slot], ksem.at[slot])

    def vcopy(i, slot):
        return pltpu.make_async_copy(v_hbm.at[i % B, i // B], vbuf.at[slot], vsem.at[slot])

    wq_c = pltpu.make_async_copy(wq_hbm, wq_v, wsem.at[0])
    wo_c = pltpu.make_async_copy(wo_hbm, wo_v, wsem.at[1])
    wg_c = pltpu.make_async_copy(wg_hbm, wg_v, wsem.at[2])
    wu_c = pltpu.make_async_copy(wu_hbm, wu_v, wsem.at[3])
    wd_c = pltpu.make_async_copy(wd_hbm, wd_v, wsem.at[4])

    wq_c.start()
    for s in range(NBUF):
        kcopy(s, s).start()
        vcopy(s, s).start()
    wo_c.start()
    wg_c.start()
    wu_c.start()
    wd_c.start()

    x = x_ref[:, 0, :]
    wq_c.wait()
    q = jnp.dot(x, wq_v[...], preferred_element_type=f32).astype(bf16)
    for h in range(H):
        q_v[h] = q[:, h * DH:(h + 1) * DH]
    acc_v[...] = jnp.zeros_like(acc_v)
    oh_v[...] = jnp.zeros_like(oh_v)

    row = jax.lax.broadcasted_iota(jnp.int32, (B, DH), 0)

    def body(i, carry):
        slot = i % NBUF
        h = i // B
        b = i % B
        kcopy(i, slot).wait()
        s = jax.lax.dot_general(q_v[h], kbuf[slot], (((1,), (1,)), ((), ())),
                                preferred_element_type=f32) * (DH ** -0.5)
        m = jnp.max(s, axis=-1, keepdims=True)
        e = jnp.exp(s - m)
        l = jnp.sum(e, axis=-1, keepdims=True)
        p = (e / l).astype(bf16)
        vcopy(i, slot).wait()
        o = jnp.dot(p, vbuf[slot], preferred_element_type=f32)

        @pl.when(i + NBUF < NPAIR)
        def _():
            kcopy(i + NBUF, slot).start()
            vcopy(i + NBUF, slot).start()

        oh = jnp.where(row == b, o, oh_v[...])
        oh_v[...] = oh

        @pl.when(i == 1)
        def _():
            wo_c.wait()

        @pl.when(b == B - 1)
        def _():
            off = pl.multiple_of(h * DH, DH)
            acc_v[...] += jnp.dot(oh.astype(bf16), wo_v[pl.ds(off, DH), :], preferred_element_type=f32)

        @pl.when(i == 16)
        def _():
            wg_c.wait()
            wu_c.wait()
            wd_c.wait()
            xf = x.astype(f32)
            r = jnp.sum(xf * wr_ref[...].astype(f32).reshape(1, D), axis=-1, keepdims=True)
            g = jnp.dot(x, wg_v[...], preferred_element_type=f32)
            u = jnp.dot(x, wu_v[...], preferred_element_type=f32)
            hmid = (jax.nn.silu(g) * u).astype(bf16)
            y = jnp.dot(hmid, wd_v[...], preferred_element_type=f32) * jax.nn.sigmoid(r)
            b_v[...] = xf + (xf * 0.0 + y)

        return carry

    jax.lax.fori_loop(0, NPAIR, body, 0)
    xf = x.astype(f32)
    gate = jax.nn.sigmoid(jnp.sum(xf * gw_ref[...].astype(f32).reshape(1, D), axis=-1, keepdims=True))
    out = gate * acc_v[...] + (1.0 - gate) * b_v[...]
    o_ref[:, 0, :] = out.astype(o_ref.dtype)


@jax.jit
def pallas_gated_mix__mha_block_cached__moe_arch_mod__decode_kernel(
        A_x, A_k_cache, A_v_cache, A_wq, A_wo, B_x, B_w_r, B_w_gate, B_w_up, B_w_down, gate_w):
    vm = pl.BlockSpec(memory_space=pltpu.VMEM)
    hbm = pl.BlockSpec(memory_space=pl.ANY)
    return pl.pallas_call(
        _kernel,
        out_shape=jax.ShapeDtypeStruct((B, 1, D), A_x.dtype),
        in_specs=[vm, vm, vm, hbm, hbm, hbm, hbm, hbm, hbm, hbm],
        out_specs=vm,
        scratch_shapes=[
            pltpu.VMEM((NBUF, SK, DH), bf16),
            pltpu.VMEM((NBUF, SK, DH), bf16),
            pltpu.VMEM((D, H * DH), bf16),
            pltpu.VMEM((H * DH, D), bf16),
            pltpu.VMEM((D, F), bf16),
            pltpu.VMEM((D, F), bf16),
            pltpu.VMEM((F, D), bf16),
            pltpu.VMEM((H, B, DH), bf16),
            pltpu.VMEM((B, DH), f32),
            pltpu.VMEM((B, D), f32),
            pltpu.VMEM((B, D), f32),
            pltpu.SemaphoreType.DMA((NBUF,)),
            pltpu.SemaphoreType.DMA((NBUF,)),
            pltpu.SemaphoreType.DMA((5,)),
        ],
        compiler_params=pltpu.CompilerParams(vmem_limit_bytes=100 * 1024 * 1024),
    )(A_x, B_w_r, gate_w, A_k_cache, A_v_cache, A_wq, A_wo, B_w_gate, B_w_up, B_w_down)
```

```python
import jax
import jax.numpy as jnp
import jax.experimental.pallas as pl
import jax.experimental.pallas.tpu as pltpu

B, D, H, SK, DH, F = 4, 1024, 32, 8192, 128, 3584
R = 512
NBUF = 4
CH = 32
NC = SK // R
NIT = H * NC
f32 = jnp.float32
bf16 = jnp.bfloat16


def _kernel(x_ref, wr_ref, gw_ref, k_hbm, v_hbm, wq_hbm, wo_hbm, wg_hbm, wu_hbm, wd_hbm,
            o_ref,
            kbuf, vbuf, wq_v, wo_v, wg_v, wu_v, wd_v, q_v, m_v, l_v, a_v, acc_v, b_v,
            ksem, vsem, wsem):
    def start_block(hbm, buf, sem, i, slot, prio):
        h = i // NC
        r0 = (i % NC) * R
        r0 = (i % NC) * (R // 2)
        for c in range(R // CH):
            pltpu.make_async_copy(
                hbm.at[:, h, pl.ds(r0 + (c // 2) * CH + (c % 2) * (SK // 2), CH), :],
                buf.at[slot, c], sem.at[slot]).start(priority=c % 2)

    def wait_block(buf, sem, slot):
        pltpu.make_async_copy(buf.at[slot], buf.at[slot], sem.at[slot]).wait()

    def start_w(hbm, buf, sem):
        _, rows, cols = hbm.shape
        cw = 0
        n = 0
        if cw == 0:
            pltpu.make_async_copy(hbm, buf, sem).start()
            return
        def body(r, c):
            r0 = pl.multiple_of(r * 16, 16)
            for j in range(cols // cw):
                pltpu.make_async_copy(hbm.at[:, pl.ds(r0, 16), pl.ds(j * cw, cw)],
                                      buf.at[:, pl.ds(r0, 16), pl.ds(j * cw, cw)], sem).start(priority=j % 2)
            return c
        jax.lax.fori_loop(0, rows // 16, body, 0)

    def wait_w(buf, sem):
        pltpu.make_async_copy(buf, buf, sem).wait()

    start_w(wq_hbm, wq_v, wsem.at[0])
    for s in range(NBUF):
        start_block(k_hbm, kbuf, ksem, s, s, 0)
        start_block(v_hbm, vbuf, vsem, s, s, 1)
    start_w(wo_hbm, wo_v, wsem.at[1])
    start_w(wg_hbm, wg_v, wsem.at[2])
    start_w(wu_hbm, wu_v, wsem.at[3])
    start_w(wd_hbm, wd_v, wsem.at[4])

    x = x_ref[:, 0, :]
    xf = x.astype(f32)

    def xdot(w_v):
        kq = w_v.shape[1]
        out = None
        for j in range(4):
            t = jnp.dot(x[:, j * kq:(j + 1) * kq], w_v[j], preferred_element_type=f32)
            out = t if out is None else out + t
        return out

    wait_w(wq_v, wsem.at[0])
    q = xdot(wq_v).astype(bf16)
    for h in range(H):
        q_v[h] = q[:, h * DH:(h + 1) * DH]
    acc_v[...] = jnp.zeros_like(acc_v)
    m_v[...] = jnp.full_like(m_v, -jnp.inf)
    l_v[...] = jnp.zeros_like(l_v)
    a_v[...] = jnp.zeros_like(a_v)

    wait_w(wo_v, wsem.at[1])
    wait_w(wg_v, wsem.at[2])
    wait_w(wu_v, wsem.at[3])
    wait_w(wd_v, wsem.at[4])
    r = jnp.sum(xf * wr_ref[...].astype(f32).reshape(1, D), axis=-1, keepdims=True)
    g = xdot(wg_v)
    u = xdot(wu_v)
    hmid = (jax.nn.silu(g) * u).astype(bf16)
    y = None
    for j in range(4):
        t = jnp.dot(hmid[:, j * (F // 4):(j + 1) * (F // 4)], wd_v[j], preferred_element_type=f32)
        y = t if y is None else y + t
    y = y * jax.nn.sigmoid(r)
    b_v[...] = xf + (xf * 0.0 + y)

    def body(i, carry):
        slot = i % NBUF
        h = i // NC
        c = i % NC
        qh = q_v[h]
        wait_block(kbuf, ksem, slot)
        rows = jax.lax.broadcasted_iota(jnp.int32, (B, R), 0)
        s = None
        for b in range(B):
            sb = jax.lax.dot_general(qh, kbuf[slot, :, b].reshape(R, DH), (((1,), (1,)), ((), ())),
                                     preferred_element_type=f32)
            s = sb if s is None else jnp.where(rows == b, sb, s)
        s = s * (DH ** -0.5)

        @pl.when(i + NBUF < NIT)
        def _():
            start_block(k_hbm, kbuf, ksem, i + NBUF, slot, 0)

        m_old = m_v[...]
        m_new = jnp.maximum(m_old, jnp.max(s, axis=-1, keepdims=True))
        alpha = jnp.exp(m_old - m_new)
        e = jnp.exp(s - m_new)
        l_new = alpha * l_v[...] + jnp.sum(e, axis=-1, keepdims=True)
        p = e.astype(bf16)
        wait_block(vbuf, vsem, slot)
        rows2 = jax.lax.broadcasted_iota(jnp.int32, (B, DH), 0)
        o = None
        for b in range(B):
            ob = jnp.dot(p, vbuf[slot, :, b].reshape(R, DH), preferred_element_type=f32)
            o = ob if o is None else jnp.where(rows2 == b, ob, o)

        @pl.when(i + NBUF < NIT)
        def _():
            start_block(v_hbm, vbuf, vsem, i + NBUF, slot, 1)

        a_new = alpha * a_v[...] + o
        m_v[...] = m_new
        l_v[...] = l_new
        a_v[...] = a_new

        @pl.when(c == NC - 1)
        def _():
            oh = (a_new / l_new).astype(bf16)
            off = pl.multiple_of((h % 8) * DH, DH)
            acc_v[...] += jnp.dot(oh, wo_v[h // 8, pl.ds(off, DH), :], preferred_element_type=f32)
            m_v[...] = jnp.full_like(m_v, -jnp.inf)
            l_v[...] = jnp.zeros_like(l_v)
            a_v[...] = jnp.zeros_like(a_v)

        return carry

    jax.lax.fori_loop(0, NIT, body, 0)
    gate = jax.nn.sigmoid(jnp.sum(xf * gw_ref[...].astype(f32).reshape(1, D), axis=-1, keepdims=True))
    out = gate * acc_v[...] + (1.0 - gate) * b_v[...]
    o_ref[:, 0, :] = out.astype(o_ref.dtype)


@jax.jit
def pallas_gated_mix__mha_block_cached__moe_arch_mod__decode_kernel(
        A_x, A_k_cache, A_v_cache, A_wq, A_wo, B_x, B_w_r, B_w_gate, B_w_up, B_w_down, gate_w):
    vm = pl.BlockSpec(memory_space=pltpu.VMEM)
    hbm = pl.BlockSpec(memory_space=pl.ANY)
    split = lambda w: w.reshape(4, w.shape[0] // 4, w.shape[1])
    return pl.pallas_call(
        _kernel,
        out_shape=jax.ShapeDtypeStruct((B, 1, D), A_x.dtype),
        in_specs=[vm, vm, vm, hbm, hbm, hbm, hbm, hbm, hbm, hbm],
        out_specs=vm,
        scratch_shapes=[
            pltpu.VMEM((NBUF, R // CH, B, CH, DH), bf16),
            pltpu.VMEM((NBUF, R // CH, B, CH, DH), bf16),
            pltpu.VMEM((4, D // 4, H * DH), bf16),
            pltpu.VMEM((4, H * DH // 4, D), bf16),
            pltpu.VMEM((4, D // 4, F), bf16),
            pltpu.VMEM((4, D // 4, F), bf16),
            pltpu.VMEM((4, F // 4, D), bf16),
            pltpu.VMEM((H, B, DH), bf16),
            pltpu.VMEM((B, 1), f32),
            pltpu.VMEM((B, 1), f32),
            pltpu.VMEM((B, DH), f32),
            pltpu.VMEM((B, D), f32),
            pltpu.VMEM((B, D), f32),
            pltpu.SemaphoreType.DMA((NBUF,)),
            pltpu.SemaphoreType.DMA((NBUF,)),
            pltpu.SemaphoreType.DMA((5,)),
        ],
        compiler_params=pltpu.CompilerParams(vmem_limit_bytes=110 * 1024 * 1024),
    )(A_x, B_w_r, gate_w, A_k_cache, A_v_cache, split(A_wq), split(A_wo), split(B_w_gate), split(B_w_up), split(B_w_down))
```

```python
import jax
import jax.numpy as jnp
import jax.experimental.pallas as pl
import jax.experimental.pallas.tpu as pltpu

B, D, H, SK, DH, F = 4, 1024, 32, 8192, 128, 3584
R = 512
NBUF = 4
CH = 32
WR = 128
HALF = 'b2'
NC = SK // R
NIT = H * NC
f32 = jnp.float32
bf16 = jnp.bfloat16


def _kernel(x_hbm, wr_hbm, gw_hbm, k_hbm, v_hbm, wq_hbm, wo_hbm, wg_hbm, wu_hbm, wd_hbm,
            o_ref,
            x_v, wr_v, gw_v, kbuf, vbuf, wq_v, wo_v, wg_v, wu_v, wd_v, q_v, m_v, l_v, a_v, acc_v, b_v,
            ksem, vsem, wsem):
    def start_block(hbm, buf, sem, i, slot):
        h = i // NC
        c0 = i % NC
        for c in range(R // CH):
            if HALF == "half":
                r0 = c0 * (R // 2) + (c // 2) * CH + (c % 2) * (SK // 2)
                src = hbm.at[:, h, pl.ds(r0, CH), :]
                dst = buf.at[slot, c]
            elif HALF == "blk":
                r0 = c0 * R + (c // 2) * CH + (c % 2) * (R // 2)
                src = hbm.at[:, h, pl.ds(r0, CH), :]
                dst = buf.at[slot, c]
            elif HALF == "seq":
                r0 = c0 * R + c * CH
                src = hbm.at[:, h, pl.ds(r0, CH), :]
                dst = buf.at[slot, c]
            elif HALF == "b2":
                r0 = c0 * R + (c // 2) * 2 * CH
                src = hbm.at[pl.ds(2 * (c % 2), 2), h, pl.ds(r0, 2 * CH), :]
                dst = buf.at[slot, c // 2, pl.ds(2 * (c % 2), 2)]
            elif HALF == "b1":
                r0 = c0 * R + (c // 4) * 4 * CH
                src = hbm.at[c % 4, h, pl.ds(r0, 4 * CH), :]
                dst = buf.at[slot, c // 4, c % 4]
            pltpu.make_async_copy(src, dst, sem.at[slot]).start(priority=c % 2)

    def wait_block(buf, sem, slot):
        pltpu.make_async_copy(buf.at[slot], buf.at[slot], sem.at[slot]).wait()

    def start_w(hbm, buf, sem):
        rows, cols = hbm.shape
        def body(r, c):
            r0 = pl.multiple_of(r * WR, WR)
            for j in range(cols // 128):
                pltpu.make_async_copy(hbm.at[pl.ds(r0, WR), pl.ds(j * 128, 128)],
                                      buf.at[j, pl.ds(r0, WR), :], sem).start(priority=j % 2)
            return c
        jax.lax.fori_loop(0, rows // WR, body, 0)

    def wait_w(buf, sem):
        pltpu.make_async_copy(buf, buf, sem).wait()

    x_c = pltpu.make_async_copy(x_hbm, x_v, wsem.at[5])
    wr_c = pltpu.make_async_copy(wr_hbm, wr_v, wsem.at[6])
    gw_c = pltpu.make_async_copy(gw_hbm, gw_v, wsem.at[7])
    start_w(wq_hbm, wq_v, wsem.at[0])
    x_c.start()
    wr_c.start()
    gw_c.start()
    for s in range(NBUF):
        start_block(k_hbm, kbuf, ksem, s, s)
        start_block(v_hbm, vbuf, vsem, s, s)
    start_w(wo_hbm, wo_v, wsem.at[1])
    start_w(wg_hbm, wg_v, wsem.at[2])
    start_w(wu_hbm, wu_v, wsem.at[3])
    start_w(wd_hbm, wd_v, wsem.at[4])

    x_c.wait()
    wr_c.wait()
    gw_c.wait()
    x = x_v[...]
    xf = x.astype(f32)

    wait_w(wq_v, wsem.at[0])
    for h in range(H):
        q_v[h] = jnp.dot(x, wq_v[h], preferred_element_type=f32).astype(bf16)
    acc_v[...] = jnp.zeros_like(acc_v)
    m_v[...] = jnp.full_like(m_v, -jnp.inf)
    l_v[...] = jnp.zeros_like(l_v)
    a_v[...] = jnp.zeros_like(a_v)

    def ffn():
        wait_w(wo_v, wsem.at[1])
        wait_w(wg_v, wsem.at[2])
        wait_w(wu_v, wsem.at[3])
        wait_w(wd_v, wsem.at[4])
        r = jnp.sum(xf * wr_v[...].astype(f32).reshape(1, D), axis=-1, keepdims=True)
        g = jnp.concatenate([jnp.dot(x, wg_v[j], preferred_element_type=f32) for j in range(F // 128)], axis=1)
        u = jnp.concatenate([jnp.dot(x, wu_v[j], preferred_element_type=f32) for j in range(F // 128)], axis=1)
        hmid = (jax.nn.silu(g) * u).astype(bf16)
        y = jnp.concatenate([jnp.dot(hmid, wd_v[j], preferred_element_type=f32) for j in range(D // 128)], axis=1)
        y = y * jax.nn.sigmoid(r)
        b_v[...] = xf + (xf * 0.0 + y)

    gate = jax.nn.sigmoid(jnp.sum(xf * gw_v[...].astype(f32).reshape(1, D), axis=-1, keepdims=True))

    def body(i, carry):
        slot = i % NBUF
        h = i // NC
        c = i % NC
        qh = q_v[h]
        wait_block(kbuf, ksem, slot)
        rows = jax.lax.broadcasted_iota(jnp.int32, (B, R), 0)
        s = None
        for b in range(B):
            sb = jax.lax.dot_general(qh, kbuf[slot, :, b].reshape(R, DH), (((1,), (1,)), ((), ())),
                                     preferred_element_type=f32)
            s = sb if s is None else jnp.where(rows == b, sb, s)
        s = s * (DH ** -0.5)

        @pl.when(i + NBUF < NIT)
        def _():
            start_block(k_hbm, kbuf, ksem, i + NBUF, slot)

        m_old = m_v[...]
        m_new = jnp.maximum(m_old, jnp.max(s, axis=-1, keepdims=True))
        alpha = jnp.exp(m_old - m_new)
        e = jnp.exp(s - m_new)
        l_new = alpha * l_v[...] + jnp.sum(e, axis=-1, keepdims=True)
        p = e.astype(bf16)
        wait_block(vbuf, vsem, slot)
        rows2 = jax.lax.broadcasted_iota(jnp.int32, (B, DH), 0)
        o = None
        for b in range(B):
            ob = jnp.dot(p, vbuf[slot, :, b].reshape(R, DH), preferred_element_type=f32)
            o = ob if o is None else jnp.where(rows2 == b, ob, o)

        @pl.when(i + NBUF < NIT)
        def _():
            start_block(v_hbm, vbuf, vsem, i + NBUF, slot)

        a_new = alpha * a_v[...] + o
        m_v[...] = m_new
        l_v[...] = l_new
        a_v[...] = a_new

        pl.when(i == NBUF)(ffn)

        @pl.when(c == NC - 1)
        def _():
            oh = (a_new / l_new).astype(bf16)
            off = pl.multiple_of(h * DH, DH)
            acc_v[...] += jnp.concatenate(
                [jnp.dot(oh, wo_v[j, pl.ds(off, DH), :], preferred_element_type=f32) for j in range(D // 128)], axis=1)
            m_v[...] = jnp.full_like(m_v, -jnp.inf)
            l_v[...] = jnp.zeros_like(l_v)
            a_v[...] = jnp.zeros_like(a_v)

        return carry

    jax.lax.fori_loop(0, NIT, body, 0)
    out = gate * acc_v[...] + (1.0 - gate) * b_v[...]
    o_ref[...] = out.astype(o_ref.dtype)


@jax.jit
def pallas_gated_mix__mha_block_cached__moe_arch_mod__decode_kernel(
        A_x, A_k_cache, A_v_cache, A_wq, A_wo, B_x, B_w_r, B_w_gate, B_w_up, B_w_down, gate_w):
    vm = pl.BlockSpec(memory_space=pltpu.VMEM)
    hbm = pl.BlockSpec(memory_space=pl.ANY)
    g = {"b2": 2, "b1": 4}.get(HALF, 1)
    out = pl.pallas_call(
        _kernel,
        out_shape=jax.ShapeDtypeStruct((B, D), A_x.dtype),
        in_specs=[hbm] * 10,
        out_specs=vm,
        scratch_shapes=[
            pltpu.VMEM((B, D), bf16),
            pltpu.VMEM((D,), bf16),
            pltpu.VMEM((D,), bf16),
            pltpu.VMEM((NBUF, R // CH // g, B, CH * g, DH), bf16),
            pltpu.VMEM((NBUF, R // CH // g, B, CH * g, DH), bf16),
            pltpu.VMEM((H, D, 128), bf16),
            pltpu.VMEM((D // 128, H * DH, 128), bf16),
            pltpu.VMEM((F // 128, D, 128), bf16),
            pltpu.VMEM((F // 128, D, 128), bf16),
            pltpu.VMEM((D // 128, F, 128), bf16),
            pltpu.VMEM((H, B, DH), bf16),
            pltpu.VMEM((B, 1), f32),
            pltpu.VMEM((B, 1), f32),
            pltpu.VMEM((B, DH), f32),
            pltpu.VMEM((B, D), f32),
            pltpu.VMEM((B, D), f32),
            pltpu.SemaphoreType.DMA((NBUF,)),
            pltpu.SemaphoreType.DMA((NBUF,)),
            pltpu.SemaphoreType.DMA((8,)),
        ],
        compiler_params=pltpu.CompilerParams(vmem_limit_bytes=110 * 1024 * 1024),
    )(A_x.reshape(B, D), B_w_r, gate_w, A_k_cache, A_v_cache, A_wq, A_wo, B_w_gate, B_w_up, B_w_down)
    return out.reshape(B, 1, D)
```

```python
import jax
import jax.numpy as jnp
import jax.experimental.pallas as pl
import jax.experimental.pallas.tpu as pltpu

B, D, H, SK, DH, F = 4, 1024, 32, 8192, 128, 3584
R = 512
NBUF = 12
CH = 32
WR = 128
WMODE = 'col'
NC = SK // R
f32 = jnp.float32
bf16 = jnp.bfloat16


def _kernel(x_hbm, wr_hbm, gw_hbm, k_hbm, v_hbm, wq_hbm, wo_hbm, wg_hbm, wu_hbm, wd_hbm,
            o_ref,
            x_v, wr_v, gw_v, ring, wq_v, wo_v, wg_v, wu_v, wd_v, q_v, s_v, b_v,
            rsem, wsem):
    def start_block(hbm, h, c0, slot):
        for c in range(R // CH):
            r0 = c0 * (R // 2) + (c // 2) * CH + (c % 2) * (SK // 2)
            pltpu.make_async_copy(hbm.at[:, h, pl.ds(r0, CH), :], ring.at[slot, c],
                                  rsem.at[slot]).start(priority=c % 2)

    def wait_block(slot):
        pltpu.make_async_copy(ring.at[slot], ring.at[slot], rsem.at[slot]).wait()

    def start_w(hbm, buf, sem):
        rows, cols = hbm.shape
        if WMODE == "col":
            def body(r, c):
                r0 = pl.multiple_of(r * WR, WR)
                for j in range(cols // 128):
                    pltpu.make_async_copy(hbm.at[pl.ds(r0, WR), pl.ds(j * 128, 128)],
                                          buf.at[j, pl.ds(r0, WR), :], sem).start(priority=j % 2)
                return c
            jax.lax.fori_loop(0, rows // WR, body, 0)
        elif WMODE == "half":
            def body(r, c):
                for j in range(cols // 128):
                    for p in range(2):
                        r0 = pl.multiple_of(r * WR + p * (rows // 2), WR)
                        pltpu.make_async_copy(hbm.at[pl.ds(r0, WR), pl.ds(j * 128, 128)],
                                              buf.at[j, pl.ds(r0, WR), :], sem).start(priority=p)
                return c
            jax.lax.fori_loop(0, rows // WR // 2, body, 0)

    def wait_w(buf, sem):
        pltpu.make_async_copy(buf, buf, sem).wait()

    x_c = pltpu.make_async_copy(x_hbm, x_v, wsem.at[5])
    wr_c = pltpu.make_async_copy(wr_hbm, wr_v, wsem.at[6])
    gw_c = pltpu.make_async_copy(gw_hbm, gw_v, wsem.at[7])
    start_w(wq_hbm, wq_v, wsem.at[0])
    x_c.start()
    wr_c.start()
    gw_c.start()

    def first(s, c):
        start_block(k_hbm, 0, s, s)
        return c
    jax.lax.fori_loop(0, NBUF, first, 0)
    start_w(wo_hbm, wo_v, wsem.at[1])
    start_w(wg_hbm, wg_v, wsem.at[2])
    start_w(wu_hbm, wu_v, wsem.at[3])
    start_w(wd_hbm, wd_v, wsem.at[4])

    x_c.wait()
    wr_c.wait()
    gw_c.wait()
    x = x_v[...]
    xf = x.astype(f32)

    wait_w(wq_v, wsem.at[0])
    for h in range(H):
        q_v[h] = jnp.dot(x, wq_v[h], preferred_element_type=f32).astype(bf16)

    def ffn():
        wait_w(wo_v, wsem.at[1])
        wait_w(wg_v, wsem.at[2])
        wait_w(wu_v, wsem.at[3])
        wait_w(wd_v, wsem.at[4])
        r = jnp.sum(xf * wr_v[...].astype(f32).reshape(1, D), axis=-1, keepdims=True)
        g = jnp.concatenate([jnp.dot(x, wg_v[j], preferred_element_type=f32) for j in range(F // 128)], axis=1)
        u = jnp.concatenate([jnp.dot(x, wu_v[j], preferred_element_type=f32) for j in range(F // 128)], axis=1)
        hmid = (jax.nn.silu(g) * u).astype(bf16)
        y = jnp.concatenate([jnp.dot(hmid, wd_v[j], preferred_element_type=f32) for j in range(D // 128)], axis=1)
        y = y * jax.nn.sigmoid(r)
        b_v[...] = xf + (xf * 0.0 + y)

    rows_s = jax.lax.broadcasted_iota(jnp.int32, (B, R), 0)
    rows_o = jax.lax.broadcasted_iota(jnp.int32, (B, DH), 0)

    def head(h, carry):
        acc, slot0 = carry
        qh = q_v[h]

        def kstep(c, carry):
            mv, slot = carry
            wait_block(slot)
            s = None
            for b in range(B):
                sb = jax.lax.dot_general(qh, ring[slot, :, b].reshape(R, DH), (((1,), (1,)), ((), ())),
                                         preferred_element_type=f32)
                s = sb if s is None else jnp.where(rows_s == b, sb, s)
            s = s * (DH ** -0.5)

            @pl.when(c + NBUF < NC)
            def _():
                start_block(k_hbm, h, c + NBUF, slot)

            @pl.when(c + NBUF >= NC)
            def _():
                start_block(v_hbm, h, c + NBUF - NC, slot)

            s_v[c] = s
            return jnp.maximum(mv, s), jnp.where(slot == NBUF - 1, 0, slot + 1)

        mv, slot0 = jax.lax.fori_loop(0, NC, kstep, (jnp.full((B, R), -jnp.inf, f32), slot0))
        m = jnp.max(mv, axis=-1, keepdims=True)

        pl.when(h == 0)(ffn)

        def vstep(c, carry):
            lv, o_acc, slot = carry
            e = jnp.exp(s_v[c] - m)
            p = e.astype(bf16)
            wait_block(slot)
            o = None
            for b in range(B):
                ob = jnp.dot(p, ring[slot, :, b].reshape(R, DH), preferred_element_type=f32)
                o = ob if o is None else jnp.where(rows_o == b, ob, o)

            @pl.when(c + NBUF < NC)
            def _():
                start_block(v_hbm, h, c + NBUF, slot)

            @pl.when(jnp.logical_and(c + NBUF >= NC, h + 1 < H))
            def _():
                start_block(k_hbm, h + 1, c + NBUF - NC, slot)

            return lv + e, o_acc + o, jnp.where(slot == NBUF - 1, 0, slot + 1)

        lv, o_acc, slot0 = jax.lax.fori_loop(
            0, NC, vstep, (jnp.zeros((B, R), f32), jnp.zeros((B, DH), f32), slot0))
        oh = (o_acc / jnp.sum(lv, axis=-1, keepdims=True)).astype(bf16)
        off = pl.multiple_of(h * DH, DH)
        acc = acc + jnp.concatenate(
            [jnp.dot(oh, wo_v[j, pl.ds(off, DH), :], preferred_element_type=f32) for j in range(D // 128)], axis=1)
        return acc, slot0

    acc, _ = jax.lax.fori_loop(0, H, head, (jnp.zeros((B, D), f32), jnp.int32(0)))
    gate = jax.nn.sigmoid(jnp.sum(xf * gw_v[...].astype(f32).reshape(1, D), axis=-1, keepdims=True))
    out = gate * acc + (1.0 - gate) * b_v[...]
    o_ref[...] = out.astype(o_ref.dtype)


@jax.jit
def pallas_gated_mix__mha_block_cached__moe_arch_mod__decode_kernel(
        A_x, A_k_cache, A_v_cache, A_wq, A_wo, B_x, B_w_r, B_w_gate, B_w_up, B_w_down, gate_w):
    vm = pl.BlockSpec(memory_space=pltpu.VMEM)
    hbm = pl.BlockSpec(memory_space=pl.ANY)
    out = pl.pallas_call(
        _kernel,
        out_shape=jax.ShapeDtypeStruct((B, D), A_x.dtype),
        in_specs=[hbm] * 10,
        out_specs=vm,
        scratch_shapes=[
            pltpu.VMEM((B, D), bf16),
            pltpu.VMEM((D,), bf16),
            pltpu.VMEM((D,), bf16),
            pltpu.VMEM((NBUF, R // CH, B, CH, DH), bf16),
            pltpu.VMEM((H, D, 128), bf16),
            pltpu.VMEM((D // 128, H * DH, 128), bf16),
            pltpu.VMEM((F // 128, D, 128), bf16),
            pltpu.VMEM((F // 128, D, 128), bf16),
            pltpu.VMEM((D // 128, F, 128), bf16),
            pltpu.VMEM((H, B, DH), bf16),
            pltpu.VMEM((NC, B, R), f32),
            pltpu.VMEM((B, D), f32),
            pltpu.SemaphoreType.DMA((NBUF,)),
            pltpu.SemaphoreType.DMA((8,)),
        ],
        compiler_params=pltpu.CompilerParams(vmem_limit_bytes=110 * 1024 * 1024),
    )(A_x.reshape(B, D), B_w_r, gate_w, A_k_cache, A_v_cache, A_wq, A_wo, B_w_gate, B_w_up, B_w_down)
    return out.reshape(B, 1, D)
```

```python
import jax
import jax.numpy as jnp
import jax.experimental.pallas as pl
import jax.experimental.pallas.tpu as pltpu

B, D, H, SK, DH, F = 4, 1024, 32, 8192, 128, 3584
R = 512
NC = SK // R
CH = 32
WC = 512
f32 = jnp.float32
bf16 = jnp.bfloat16


def _kernel(x_hbm, wr_hbm, gw_hbm, k_hbm, v_hbm, wq_hbm, wo_hbm, wg_hbm, wu_hbm, wd_hbm,
            o_ref,
            x_v, wr_v, gw_v, ring, wq_v, wo_v, wg_v, wu_v, wd_v, q_v, s_v, b_v,
            rsem, wsem):
    def start_block(hbm, h, c):
        for n in range(R // CH):
            r0 = c * (R // 2) + (n // 2) * CH + (n % 2) * (SK // 2)
            pltpu.make_async_copy(hbm.at[:, h, pl.ds(r0, CH), :], ring.at[c, n],
                                  rsem.at[c]).start(priority=n % 2)

    def wait_block(c):
        pltpu.make_async_copy(ring.at[c], ring.at[c], rsem.at[c]).wait()

    def start_w(hbm, buf, sem):
        _, nr, _, cols = hbm.shape

        def body(r, carry):
            for j in range(cols // WC):
                for p in range(2):
                    idx = (slice(None), r + p * (nr // 2), slice(None), pl.ds(j * WC, WC))
                    pltpu.make_async_copy(hbm.at[idx], buf.at[idx], sem).start(priority=p)
            return carry

        jax.lax.fori_loop(0, nr // 2, body, 0)

    def wait_w(buf, sem):
        pltpu.make_async_copy(buf, buf, sem).wait()

    def wdot(lhs, w_v):
        _, nr, _, cols = w_v.shape
        return [jnp.dot(lhs, w_v[:, :, :, pl.ds(j * 128, 128)].reshape(32 * nr, 128),
                        preferred_element_type=f32) for j in range(cols // 128)]

    small = [pltpu.make_async_copy(src, dst, wsem.at[5 + i])
             for i, (src, dst) in enumerate(((x_hbm, x_v), (wr_hbm, wr_v), (gw_hbm, gw_v)))]

    start_w(wq_hbm, wq_v, wsem.at[0])
    for cp in small:
        cp.start()

    def first(c, carry):
        start_block(k_hbm, 0, c)
        return carry

    jax.lax.fori_loop(0, NC, first, 0)

    for cp in small:
        cp.wait()
    x = x_v[...]
    xf = x.astype(f32)

    wait_w(wq_v, wsem.at[0])
    for h, qh in enumerate(wdot(x, wq_v)):
        q_v[h] = qh.astype(bf16)

    start_w(wo_hbm, wo_v, wsem.at[1])
    start_w(wg_hbm, wg_v, wsem.at[2])
    start_w(wu_hbm, wu_v, wsem.at[3])
    start_w(wd_hbm, wd_v, wsem.at[4])

    def ffn():
        wait_w(wo_v, wsem.at[1])
        wait_w(wg_v, wsem.at[2])
        wait_w(wu_v, wsem.at[3])
        wait_w(wd_v, wsem.at[4])
        r = jnp.sum(xf * wr_v[...].astype(f32).reshape(1, D), axis=-1, keepdims=True)
        g = jnp.concatenate(wdot(x, wg_v), axis=1)
        u = jnp.concatenate(wdot(x, wu_v), axis=1)
        hmid = (jax.nn.silu(g) * u).astype(bf16)
        y = jnp.concatenate(wdot(hmid, wd_v), axis=1) * jax.nn.sigmoid(r)
        b_v[...] = xf + (xf * 0.0 + y)

    rows_s = jax.lax.broadcasted_iota(jnp.int32, (B, R), 0)
    rows_o = jax.lax.broadcasted_iota(jnp.int32, (B, DH), 0)

    def head(h, acc):
        qh = q_v[h]

        def kstep(c, mv):
            wait_block(c)
            s = None
            for b in range(B):
                sb = jax.lax.dot_general(qh, ring[c, :, b].reshape(R, DH), (((1,), (1,)), ((), ())),
                                         preferred_element_type=f32)
                s = sb if s is None else jnp.where(rows_s == b, sb, s)
            s = s * (DH ** -0.5)
            pl.when(h < H)(lambda: start_block(v_hbm, h, c))
            s_v[c] = s
            return jnp.maximum(mv, s)

        mv = jax.lax.fori_loop(0, NC, kstep, jnp.full((B, R), -jnp.inf, f32))
        m = jnp.max(mv, axis=-1, keepdims=True)

        pl.when(h == 0)(ffn)

        def vstep(c, carry):
            lv, o_acc = carry
            e = jnp.exp(s_v[c] - m)
            p = e.astype(bf16)
            wait_block(c)
            o = None
            for b in range(B):
                ob = jnp.dot(p, ring[c, :, b].reshape(R, DH), preferred_element_type=f32)
                o = ob if o is None else jnp.where(rows_o == b, ob, o)

            @pl.when(h + 1 < H)
            def _():
                start_block(k_hbm, h + 1, c)

            return lv + e, o_acc + o

        lv, o_acc = jax.lax.fori_loop(0, NC, vstep, (jnp.zeros((B, R), f32), jnp.zeros((B, DH), f32)))
        oh = (o_acc / jnp.sum(lv, axis=-1, keepdims=True)).astype(bf16)
        wo_h = wo_v[h // 8, pl.ds((h % 8) * 16, 16)].reshape(DH, D)
        return acc + jnp.dot(oh, wo_h, preferred_element_type=f32)

    gate = jax.nn.sigmoid(jnp.sum(xf * gw_v[...].astype(f32).reshape(1, D), axis=-1, keepdims=True))
    acc = jax.lax.fori_loop(0, H, head, jnp.zeros((B, D), f32))
    o_ref[...] = (gate * acc + (1.0 - gate) * b_v[...]).astype(o_ref.dtype)


@jax.jit
def pallas_gated_mix__mha_block_cached__moe_arch_mod__decode_kernel(
        A_x, A_k_cache, A_v_cache, A_wq, A_wo, B_x, B_w_r, B_w_gate, B_w_up, B_w_down, gate_w):
    del B_x
    weights = [w.reshape(4, w.shape[0] // 32, 8, w.shape[1])
               for w in (A_wq, A_wo, B_w_gate, B_w_up, B_w_down)]
    out = pl.pallas_call(
        _kernel,
        out_shape=jax.ShapeDtypeStruct((B, D), A_x.dtype),
        in_specs=[pl.BlockSpec(memory_space=pl.ANY)] * 10,
        out_specs=pl.BlockSpec(memory_space=pltpu.VMEM),
        scratch_shapes=[
            pltpu.VMEM((B, D), bf16),
            pltpu.VMEM((D,), bf16),
            pltpu.VMEM((D,), bf16),
            pltpu.VMEM((NC, R // CH, B, CH, DH), bf16),
            *[pltpu.VMEM(w.shape, bf16) for w in weights],
            pltpu.VMEM((H, B, DH), bf16),
            pltpu.VMEM((NC, B, R), f32),
            pltpu.VMEM((B, D), f32),
            pltpu.SemaphoreType.DMA((NC,)),
            pltpu.SemaphoreType.DMA((8,)),
        ],
        compiler_params=pltpu.CompilerParams(vmem_limit_bytes=100 * 1024 * 1024),
    )(A_x.reshape(B, D), B_w_r, gate_w, A_k_cache, A_v_cache, *weights)
    return out.reshape(B, 1, D)
```
